```python
import os as _os
_os.environ.setdefault("JAX_PLATFORMS", "cpu")
import jax
import jax.numpy as jnp

def _softmax(x, axis=-1):
    return jax.nn.softmax(x, axis=axis)
def _gelu(x):
    return jax.nn.gelu(x, approximate=True)
def _silu(x):
    return jax.nn.silu(x)
def _sigmoid(x):
    return jax.nn.sigmoid(x)
def _layernorm(x, axis=-1, eps=1e-5):
    m = jnp.mean(x, axis=axis, keepdims=True)
    v = jnp.var(x, axis=axis, keepdims=True)
    return (x - m) / jnp.sqrt(v + eps)
def _scatter_add(tgt, idx, src, axis=0):
    return tgt.at[idx].add(src)
def _segment_sum(src, seg, n):
    return jax.ops.segment_sum(src, seg, n)
class _Rng:
    def __init__(self, key):
        self._k = key
    def _next(self):
        self._k, sub = jax.random.split(self._k)
        return sub
    def normal(self, shape):
        return jax.random.normal(self._next(), shape, dtype=jnp.bfloat16)
    def randint(self, lo, hi, shape):
        return jax.random.randint(self._next(), shape, lo, hi, dtype=jnp.int32)
    def uniform(self, shape, lo=0.0, hi=1.0):
        return jax.random.uniform(self._next(), shape, jnp.bfloat16, lo, hi)
    def permutation(self, n):
        return jax.random.permutation(self._next(), n)


kernel_name = 'interleave_layers__mha_block__dense_activation_mish__prompt'

def setup_inputs():
    _rng = _Rng(jax.random.key(int.from_bytes(__import__("os").urandom(4), "little")))
    _w = (lambda a: (lambda t: t.astype(jnp.bfloat16) if jnp.issubdtype(t.dtype, jnp.floating) else t)(jnp.asarray(a)))
    def _A_setup():
        B, S, D, H = 1, 2048, 512, 32
        return {
            "x": _w((lambda *s: _rng.normal(s) * 0.05)(B, S, D)),
            "wqkv": _w((lambda *s: _rng.normal(s) * 0.05)(D, 3 * D)),
            "wo": _w((lambda *s: _rng.normal(s) * 0.05)(D, D)),
        }
    _A_in = _A_setup()

    def _B_setup():
        B, S, D, F = 1, 2048, 512, 1792
        return {
            "x": _w((lambda *s: _rng.normal(s) * 0.05)(B, S, D)),
            "w1": _w((lambda *s: _rng.normal(s) * 0.4)(D, F) * (D ** -0.5)),
            "b1": _w((lambda *s: _rng.normal(s) * 0.4)(F)),
            "w2": _w((lambda *s: _rng.normal(s) * 0.4)(F, D) * (F ** -0.5)),
        }
    _B_in = _B_setup()

    return {
        "A_x": _A_in["x"],
        "A_wqkv": _A_in["wqkv"],
        "A_wo": _A_in["wo"],
        "B_x": _B_in["x"],
        "B_w1": _B_in["w1"],
        "B_b1": _B_in["b1"],
        "B_w2": _B_in["w2"],
    }

def reference(A_x, A_wqkv, A_wo, B_x, B_w1, B_b1, B_w2):
    def _A_ref(x, wqkv, wo):
        B, S, D = x.shape
        H = 32
        Dh = D // H
        qkv = (lambda x, *d: x.transpose(*d))((x @ wqkv).reshape(B, S, 3, H, Dh), 2, 0, 3, 1, 4)
        q, k, v = qkv[0], qkv[1], qkv[2]
        scores = jnp.einsum("bhqd,bhkd->bhqk", q, k) * (Dh ** -0.5)
        p = _softmax(scores, axis=-1)
        o = jnp.einsum("bhqk,bhkd->bhqd", p, v)
        return (lambda x, *d: x.transpose(*d))(o, 0, 2, 1, 3).reshape(B, S, D) @ wo

    def _B_ref(x, w1, b1, w2):
        h = jnp.einsum("bsd,df->bsf", x, w1) + b1
        sp = jnp.log1p(jnp.exp(-jnp.abs(h))) + jnp.where(h > 0, h, jnp.zeros_like(h))
        act = h * jnp.tanh(sp)
        return jnp.einsum("bsf,fd->bsd", act, w2)

    x = A_x
    x = x + _A_ref(_layernorm(x, axis=-1), A_wqkv, A_wo)
    x = x + _B_ref(_layernorm(x, axis=-1), B_w1, B_b1, B_w2)
    x = x + _A_ref(_layernorm(x, axis=-1), A_wqkv, A_wo)
    x = x + _B_ref(_layernorm(x, axis=-1), B_w1, B_b1, B_w2)
    return x
```

```python
import functools
import jax
import jax.numpy as jnp
from jax import lax
import jax.experimental.pallas as pl
import jax.experimental.pallas.tpu as pltpu

S, D, H, DH, F = 2048, 512, 32, 16, 1792
LOG2E = 1.4426950408889634
QSCALE = (DH ** -0.5) * LOG2E


def _ln(x):
    m = jnp.mean(x, axis=-1, keepdims=True)
    xc = x - m
    v = jnp.mean(xc * xc, axis=-1, keepdims=True)
    return xc * lax.rsqrt(v + 1e-5)


def _mish(h):
    sp = jnp.log1p(jnp.exp(-jnp.abs(h))) + jnp.maximum(h, 0.0)
    return h * jnp.tanh(sp)


def make_kernel(TQ=512, TKC=128, TM=512, U=1):
    NQ = S // TQ
    NIT = H * NQ
    NC = S // TKC

    def kernel(x_ref, wqkv_ref, wo_ref, w1_ref, b1_ref, w2_ref, o_ref,
               xs_ref, qT_ref, k_ref, vT_ref, oT_ref, s_ref, wqT_ref, wvT_ref):
        wqT_ref[...] = wqkv_ref[:, 0:D].astype(jnp.float32).T.astype(jnp.bfloat16)
        wvT_ref[...] = wqkv_ref[:, 2 * D:3 * D].astype(jnp.float32).T.astype(jnp.bfloat16)

        def qkv_block(r, xblk):
            ln = _ln(xblk).astype(jnp.bfloat16)
            kk = jnp.dot(ln, wqkv_ref[:, D:2 * D], preferred_element_type=jnp.float32).astype(jnp.bfloat16)
            for g in range(4):
                k_ref[g, r * TM:(r + 1) * TM, :] = kk[:, g * 128:(g + 1) * 128]
            nt = (((1,), (1,)), ((), ()))
            qT = lax.dot_general(wqT_ref[...], ln, nt, preferred_element_type=jnp.float32) * QSCALE
            qT = qT.astype(jnp.bfloat16)
            vT = lax.dot_general(wvT_ref[...], ln, nt, preferred_element_type=jnp.float32).astype(jnp.bfloat16)
            W = min(TM, TQ)
            for j in range(TM // W):
                c0 = r * TM + j * W
                qT_ref[c0 // TQ, :, c0 % TQ:c0 % TQ + W] = qT[:, j * W:(j + 1) * W]
            for h in range(H):
                vT_ref[h, :, r * TM:(r + 1) * TM] = vT[h * DH:(h + 1) * DH, :]

        def step(it1, it2, m2):
            do1 = it1 is not None
            do2 = it2 is not None
            if do1:
                h1 = it1 // NQ
                qb1 = it1 % NQ
                g = h1 // 8
                hh = h1 % 8
                row_head = lax.broadcasted_iota(jnp.int32, (128, TQ), 0) // DH
                qg = qT_ref[qb1, pl.ds(pl.multiple_of(g * 128, 128), 128), :]
                qm = jnp.where(row_head == hh, qg, jnp.zeros_like(qg))
            if do2:
                h2 = it2 // NQ
                qb2 = it2 % NQ
            m = None
            l = None
            acc = None
            for c in range(NC):
                if do2:
                    s = s_ref[c * TKC:(c + 1) * TKC, :]
                    p = jnp.exp2(s - m2)
                    lc = jnp.sum(p.reshape(TKC // 8, 8, TQ), axis=0)
                    l = lc if l is None else l + lc
                    a = jnp.dot(vT_ref[h2, :, c * TKC:(c + 1) * TKC], p.astype(jnp.bfloat16),
                                preferred_element_type=jnp.float32)
                    acc = a if acc is None else acc + a
                if do1:
                    s = jnp.dot(k_ref[g, c * TKC:(c + 1) * TKC, :], qm, preferred_element_type=jnp.float32)
                    s_ref[c * TKC:(c + 1) * TKC, :] = s
                    mc = jnp.max(s.reshape(TKC // 8, 8, TQ), axis=0)
                    m = mc if m is None else jnp.maximum(m, mc)
            if do2:
                lt = jnp.sum(l, axis=0, keepdims=True)
                o = acc / lt
                oT_ref[qb2, pl.ds(pl.multiple_of(h2 * DH, DH), DH), :] = o.astype(jnp.bfloat16)
            if do1:
                return jnp.max(m, axis=0, keepdims=True)
            return None

        def attention():
            m0 = step(0, None, None)

            def body(j, mm):
                for u in range(U):
                    it = U * j + u
                    mm = step(jnp.minimum(it + 1, NIT - 1), it, mm)
                return mm
            lax.fori_loop(0, NIT // U, body, m0)

        def post_block(r):
            W = min(TM, TQ)
            oT = jnp.concatenate([oT_ref[(r * TM + j * W) // TQ, :, (r * TM + j * W) % TQ:(r * TM + j * W) % TQ + W]
                                  for j in range(TM // W)], axis=1)
            o = oT.astype(jnp.float32).T.astype(jnp.bfloat16)
            x1 = xs_ref[r * TM:(r + 1) * TM, :] + jnp.dot(o, wo_ref[...], preferred_element_type=jnp.float32)
            ln = _ln(x1).astype(jnp.bfloat16)
            hh = jnp.dot(ln, w1_ref[...], preferred_element_type=jnp.float32) + b1_ref[...].astype(jnp.float32)
            act = _mish(hh).astype(jnp.bfloat16)
            x2 = x1 + jnp.dot(act, w2_ref[...], preferred_element_type=jnp.float32)
            return x2

        for r in range(S // TM):
            xb = x_ref[r * TM:(r + 1) * TM, :].astype(jnp.float32)
            xs_ref[r * TM:(r + 1) * TM, :] = xb
            qkv_block(r, xb)
        for layer in range(2):
            attention()
            for r in range(S // TM):
                x2 = post_block(r)
                if layer == 0:
                    xs_ref[r * TM:(r + 1) * TM, :] = x2
                    qkv_block(r, x2)
                else:
                    o_ref[r * TM:(r + 1) * TM, :] = x2.astype(o_ref.dtype)

    def call(A_x, A_wqkv, A_wo, B_x, B_w1, B_b1, B_w2):
        x = A_x.reshape(S, D)
        out = pl.pallas_call(
            kernel,
            out_shape=jax.ShapeDtypeStruct((S, D), jnp.bfloat16),
            scratch_shapes=[
                pltpu.VMEM((S, D), jnp.float32),
                pltpu.VMEM((NQ, D, TQ), jnp.bfloat16),
                pltpu.VMEM((4, S, 128), jnp.bfloat16),
                pltpu.VMEM((H, DH, S), jnp.bfloat16),
                pltpu.VMEM((NQ, D, TQ), jnp.bfloat16),
                pltpu.VMEM((S, TQ), jnp.float32),
                pltpu.VMEM((D, D), jnp.bfloat16),
                pltpu.VMEM((D, D), jnp.bfloat16),
            ],
            compiler_params=pltpu.CompilerParams(vmem_limit_bytes=100 * 1024 * 1024),
        )(x, A_wqkv, A_wo, B_w1, B_b1.reshape(1, F), B_w2)
        return out.reshape(1, S, D)
    return call


_call = make_kernel(TQ=512,TKC=128,TM=512)


@jax.jit
def pallas_interleave_layers__mha_block__dense_activation_mish__prompt_kernel(
    A_x: jax.Array,
    A_wqkv: jax.Array,
    A_wo: jax.Array,
    B_x: jax.Array,
    B_w1: jax.Array,
    B_b1: jax.Array,
    B_w2: jax.Array,
):
    return _call(A_x, A_wqkv, A_wo, B_x, B_w1, B_b1, B_w2)
```

```python
import jax
import jax.numpy as jnp
from jax import lax
import jax.experimental.pallas as pl
import jax.experimental.pallas.tpu as pltpu

S, D, H, DH, F = 2048, 512, 32, 16, 1792
LOG2E = 1.4426950408889634
QSCALE = (DH ** -0.5) * LOG2E

TQ = 512
TKC = 128
TM = 512
U = 8
LLAG = 2
PLAG = 3
NQ = S // TQ
NIT = H * NQ
NC = S // TKC
NR = S // TM
HU = U // NQ


def _ln(x):
    m = jnp.mean(x, axis=-1, keepdims=True)
    xc = x - m
    v = jnp.mean(xc * xc, axis=-1, keepdims=True)
    return xc * lax.rsqrt(v + 1e-5)


def _mish(h):
    sp = jnp.log1p(jnp.exp(-jnp.abs(h))) + jnp.maximum(h, 0.0)
    return h * jnp.tanh(sp)


def _tree(t, op):
    while t.shape[0] > 1:
        t = t.reshape(t.shape[0] // 2, 2, 8, TQ)
        t = op(t[:, 0], t[:, 1])
    return t[0]


def _kernel(x_hbm, wqkv_hbm, wo_hbm, w1_hbm, b1_hbm, w2_hbm, o_hbm,
            xs_ref, qT_ref, k_ref, vT_ref, oT_ref, sA_ref, sB_ref, ln_ref, wqT_ref, wvT_ref,
            x_ref, wqkv_ref, wo_ref, w1_ref, b1_ref, w2_ref, o_ref, one_ref, sem_in, sem_x, sem_o):
    rows = lambda r: slice(r * TM, (r + 1) * TM)

    cp_wqkv = pltpu.make_async_copy(wqkv_hbm, wqkv_ref, sem_in.at[0])
    cp_x = [pltpu.make_async_copy(x_hbm.at[rows(r), :], x_ref.at[rows(r), :], sem_x.at[r]) for r in range(NR)]
    cp_rest = [pltpu.make_async_copy(a, b, sem_in.at[i + 1])
               for i, (a, b) in enumerate([(wo_hbm, wo_ref), (w1_hbm, w1_ref), (b1_hbm, b1_ref), (w2_hbm, w2_ref)])]
    cp_o = [pltpu.make_async_copy(o_ref.at[rows(r), :], o_hbm.at[rows(r), :], sem_o.at[r]) for r in range(NR)]
    cp_x[0].start()
    cp_wqkv.start()
    for c in cp_x[1:]:
        c.start()
    for c in cp_rest:
        c.start()
    one_ref[0] = 1

    def head_rows(h):
        if isinstance(h, int):
            return slice(h * DH, (h + 1) * DH)
        return pl.ds(pl.multiple_of(h * DH, DH), DH)

    def qkv_block(r, first=False):
        ln = ln_ref[rows(r), :]
        kk = jnp.dot(ln, wqkv_ref[:, D:2 * D], preferred_element_type=jnp.float32).astype(jnp.bfloat16)
        for h in range(H):
            k_ref[h, rows(r), :] = kk[:, h * DH:(h + 1) * DH]
        if first:
            wqT_ref[...] = wqkv_ref[:, 0:D].astype(jnp.float32).T.astype(jnp.bfloat16)
            wvT_ref[...] = wqkv_ref[:, 2 * D:3 * D].astype(jnp.float32).T.astype(jnp.bfloat16)
        nt = (((1,), (1,)), ((), ()))
        qT = lax.dot_general(wqT_ref[...], ln, nt, preferred_element_type=jnp.float32) * QSCALE
        vT = lax.dot_general(wvT_ref[...], ln, nt, preferred_element_type=jnp.float32).astype(jnp.bfloat16)
        qT_ref[r] = qT.astype(jnp.bfloat16)
        for h in range(H):
            vT_ref[h, :, rows(r)] = vT[h * DH:(h + 1) * DH, :]

    def step(it1, it2, m2, sw_ref, sr_ref, tp):
        do1 = it1 is not None
        do2 = it2 is not None
        if do1:
            h1, qb1 = it1
            qm = qT_ref[qb1, head_rows(h1), :]
        if do2:
            h2, qb2 = it2
        m = l = acc = None
        ls = []
        mcs = []
        for c in range(NC):
            ks = slice(c * TKC, (c + 1) * TKC)
            if do1:
                s = jnp.dot(k_ref[h1, ks, :], qm, preferred_element_type=jnp.float32)
                sw_ref[ks, :] = s
                mc = _tree(s.reshape(TKC // 8, 8, TQ), jnp.maximum)
                mcs.append(mc)
                m = mc if m is None else jnp.maximum(m, mc)
            if do2:
                s = sr_ref[ks, :]
                m2c = m2
                if c - LLAG >= 0:
                    m2c = jnp.where(tp >= 0, m2c, ls[c - LLAG][0:1, :])
                if do1 and c - PLAG >= 0:
                    m2c = jnp.where(tp > -1, m2c, mcs[c - PLAG][0:1, :])
                p = jnp.exp2(s - m2c)
                lc = _tree(p.reshape(TKC // 8, 8, TQ), jnp.add)
                l = lc if l is None else l + lc
                ls.append(l)
                a = jnp.dot(vT_ref[h2, :, ks], p.astype(jnp.bfloat16), preferred_element_type=jnp.float32)
                acc = a if acc is None else acc + a
        if do2:
            lt = jnp.sum(l, axis=0, keepdims=True)
            oT_ref[qb2, head_rows(h2), :] = (acc / lt).astype(jnp.bfloat16)
        if do1:
            return jnp.max(m, axis=0, keepdims=True)
        return None

    def stage_a(r):
        o = oT_ref[r].astype(jnp.float32).T.astype(jnp.bfloat16)
        x1 = xs_ref[rows(r), :] + jnp.dot(o, wo_ref[...], preferred_element_type=jnp.float32)
        xs_ref[rows(r), :] = x1
        ln_ref[rows(r), :] = _ln(x1).astype(jnp.bfloat16)

    def stage_b(r, layer):
        hh = (jnp.dot(ln_ref[rows(r), :], w1_ref[...], preferred_element_type=jnp.float32)
              + b1_ref[...].astype(jnp.float32).reshape(1, F))
        act = _mish(hh).astype(jnp.bfloat16)
        x2 = xs_ref[rows(r), :] + jnp.dot(act, w2_ref[...], preferred_element_type=jnp.float32)
        if layer == 0:
            xs_ref[rows(r), :] = x2
            ln_ref[rows(r), :] = _ln(x2).astype(jnp.bfloat16)
        else:
            o_ref[rows(r), :] = x2.astype(o_ref.dtype)
            cp_o[r].start()

    def stage_x(r):
        cp_x[r].wait()
        xb = x_ref[rows(r), :].astype(jnp.float32)
        xs_ref[rows(r), :] = xb
        ln_ref[rows(r), :] = _ln(xb).astype(jnp.bfloat16)

    def attention():
        tp0 = one_ref[0]
        m0 = step((0, 0), None, None, sA_ref, None, tp0)

        def steps(hbase, mm, last):
            for u in range(U):
                h, qb = hbase + u // NQ, u % NQ
                nxt = (hbase + (u + 1) // NQ, (u + 1) % NQ)
                if last and u == U - 1:
                    nxt = None
                    stage_a(0)
                sw, sr = (sB_ref, sA_ref) if u % 2 == 0 else (sA_ref, sB_ref)
                tp = tp0 if isinstance(h, int) else h
                mm = step(nxt, (h, qb), mm, sw, sr, tp)
            return mm

        mlast = lax.fori_loop(0, NIT // U - 1, lambda j, mm: steps(j * HU, mm, False), m0)
        steps(H - HU, mlast, True)

    stage_x(0)
    cp_wqkv.wait()
    for r in range(NR):
        if r + 1 < NR:
            stage_x(r + 1)
        qkv_block(r, first=(r == 0))
    for c in cp_rest:
        c.wait()
    for layer in range(2):
        attention()
        for t in range(1, NR + 2):
            if t < NR:
                stage_a(t)
            if 0 <= t - 1 < NR:
                stage_b(t - 1, layer)
            if layer == 0 and 0 <= t - 2 < NR:
                qkv_block(t - 2)
    for c in cp_o:
        c.wait()


@jax.jit
def pallas_interleave_layers__mha_block__dense_activation_mish__prompt_kernel(
    A_x: jax.Array,
    A_wqkv: jax.Array,
    A_wo: jax.Array,
    B_x: jax.Array,
    B_w1: jax.Array,
    B_b1: jax.Array,
    B_w2: jax.Array,
):
    assert TM == TQ and A_x.shape == (1, S, D)
    out = pl.pallas_call(
        _kernel,
        out_shape=jax.ShapeDtypeStruct((S, D), jnp.bfloat16),
        in_specs=[pl.BlockSpec(memory_space=pl.ANY)] * 6,
        out_specs=pl.BlockSpec(memory_space=pl.ANY),
        scratch_shapes=[
            pltpu.VMEM((S, D), jnp.float32),
            pltpu.VMEM((NQ, D, TQ), jnp.bfloat16),
            pltpu.VMEM((H, S, DH), jnp.bfloat16),
            pltpu.VMEM((H, DH, S), jnp.bfloat16),
            pltpu.VMEM((NQ, D, TQ), jnp.bfloat16),
            pltpu.VMEM((S, TQ), jnp.float32),
            pltpu.VMEM((S, TQ), jnp.float32),
            pltpu.VMEM((S, D), jnp.bfloat16),
            pltpu.VMEM((D, D), jnp.bfloat16),
            pltpu.VMEM((D, D), jnp.bfloat16),
            pltpu.VMEM((S, D), jnp.bfloat16),
            pltpu.VMEM((D, 3 * D), jnp.bfloat16),
            pltpu.VMEM((D, D), jnp.bfloat16),
            pltpu.VMEM((D, F), jnp.bfloat16),
            pltpu.VMEM((F,), jnp.bfloat16),
            pltpu.VMEM((F, D), jnp.bfloat16),
            pltpu.VMEM((S, D), jnp.bfloat16),
            pltpu.SMEM((1,), jnp.int32),
            pltpu.SemaphoreType.DMA((5,)),
            pltpu.SemaphoreType.DMA((NR,)),
            pltpu.SemaphoreType.DMA((NR,)),
        ],
        compiler_params=pltpu.CompilerParams(vmem_limit_bytes=100 * 1024 * 1024),
    )(A_x.reshape(S, D), A_wqkv, A_wo, B_w1, B_b1, B_w2)
    return out.reshape(1, S, D)
```
